```python
import os as _os
_os.environ.setdefault("JAX_PLATFORMS", "cpu")
import jax
import jax.numpy as jnp

def _softmax(x, axis=-1):
    return jax.nn.softmax(x, axis=axis)
def _gelu(x):
    return jax.nn.gelu(x, approximate=True)
def _silu(x):
    return jax.nn.silu(x)
def _sigmoid(x):
    return jax.nn.sigmoid(x)
def _layernorm(x, axis=-1, eps=1e-5):
    m = jnp.mean(x, axis=axis, keepdims=True)
    v = jnp.var(x, axis=axis, keepdims=True)
    return (x - m) / jnp.sqrt(v + eps)
def _scatter_add(tgt, idx, src, axis=0):
    return tgt.at[idx].add(src)
def _segment_sum(src, seg, n):
    return jax.ops.segment_sum(src, seg, n)
class _Rng:
    def __init__(self, key):
        self._k = key
    def _next(self):
        self._k, sub = jax.random.split(self._k)
        return sub
    def normal(self, shape):
        return jax.random.normal(self._next(), shape, dtype=jnp.bfloat16)
    def randint(self, lo, hi, shape):
        return jax.random.randint(self._next(), shape, lo, hi, dtype=jnp.int32)
    def uniform(self, shape, lo=0.0, hi=1.0):
        return jax.random.uniform(self._next(), shape, jnp.bfloat16, lo, hi)
    def permutation(self, n):
        return jax.random.permutation(self._next(), n)


kernel_name = 'interleave_layers__ssm_conv_h3__linear_attn_block__prompt'

def setup_inputs():
    _rng = _Rng(jax.random.key(int.from_bytes(__import__("os").urandom(4), "little")))
    _w = (lambda a: (lambda t: t.astype(jnp.bfloat16) if jnp.issubdtype(t.dtype, jnp.floating) else t)(jnp.asarray(a)))
    def _A_setup():
        B, S, D = 1, 2048, 512
        ks = 4
        return {
            "q": _w((lambda *s: _rng.normal(s) * 0.05)(B, S, D)),
            "k": _w((lambda *s: _rng.normal(s) * 0.4)(B, S, D)),
            "v": _w((lambda *s: _rng.normal(s) * 0.4)(B, S, D)),
            "shift_k": _w((lambda *s: _rng.normal(s) * 0.4)(D, ks) * 0.5),
            "ssm_k": _w((lambda *s: _rng.normal(s) * 0.4)(D, S) * (1.0 / S ** 0.5)),
            "ssm_D": _w((lambda *s: _rng.normal(s) * 0.4)(D)),
        }
    _A_in = _A_setup()

    def _B_setup():
        B, S, D = 1, 2048, 512
        return {
            "x": _w((lambda *s: _rng.normal(s) * 0.05)(B, S, D)),
            "wqkv": _w((lambda *s: _rng.normal(s) * 0.1)(D, 3 * D)),
            "wo": _w((lambda *s: _rng.normal(s) * 0.1)(D, D)),
        }
    _B_in = _B_setup()

    return {
        "A_q": _A_in["q"],
        "A_k": _A_in["k"],
        "A_v": _A_in["v"],
        "A_shift_k": _A_in["shift_k"],
        "A_ssm_k": _A_in["ssm_k"],
        "A_ssm_D": _A_in["ssm_D"],
        "B_x": _B_in["x"],
        "B_wqkv": _B_in["wqkv"],
        "B_wo": _B_in["wo"],
    }

def reference(A_q, A_k, A_v, A_shift_k, A_ssm_k, A_ssm_D, B_x, B_wqkv, B_wo):
    def _A_ref(q, k, v, shift_k, ssm_k, ssm_D):
        B, S, D = q.shape
        ks = shift_k.shape[-1]
        k_pad = jnp.pad(k, ((0, 0), (ks - 1, 0), (0, 0)))
        k_shift = jnp.zeros_like(k)
        for t in range(ks):
            k_shift = k_shift + k_pad[:, t:t + S, :] * shift_k[:, ks - 1 - t][None, None, :]
        kv = k_shift * v
        L = 2 * S
        kv_pad = jnp.pad(kv, ((0, 0), (0, S), (0, 0)))
        kf_pad = jnp.pad(ssm_k, ((0, 0), (0, S)))
        kv_f = (lambda x, axes=(-2,-1): jnp.fft.rfft2(x.astype(jnp.float32), axes=axes))(kv_pad[:, None, :, :], axes=(1, 2))
        kf_f = (lambda x, axes=(-2,-1): jnp.fft.rfft2(x.astype(jnp.float32), axes=axes))(kf_pad[:, None, :], axes=(1, 2))
        kf_f = (lambda x, *d: x.transpose(*d))(kf_f, 1, 2, 0)
        y_f = kv_f * kf_f[None, :, :, :]
        y = (lambda x, s, axes=(-2,-1): jnp.fft.irfft2(x, s=s, axes=axes).astype(jnp.bfloat16))(y_f, (1, L), axes=(1, 2))[:, 0, :S, :]
        y = y + kv * ssm_D[None, None, :]
        return q * y

    def _B_ref(x, wqkv, wo):
        B, S, D = x.shape
        H = 32; Dh = D // H
        qkv = (lambda x, *d: x.transpose(*d))((x @ wqkv).reshape(B, S, 3, H, Dh), 2, 0, 3, 1, 4)
        q, k, v = qkv[0], qkv[1], qkv[2]
        phi = lambda t: jnp.where(t > 0, t + 1, jnp.exp(t)) + 1e-6
        pq, pk = phi(q), phi(k)
        kv = jnp.einsum("bhsd,bhse->bhde", pk, v)
        z = jnp.einsum("bhsd->bhd", pk)
        num = jnp.einsum("bhqd,bhde->bhqe", pq, kv)
        den = jnp.einsum("bhqd,bhd->bhq", pq, z)[..., None] + 1e-6
        o = num / den
        return (lambda x, *d: x.transpose(*d))(o, 0, 2, 1, 3).reshape(B, S, D) @ wo

    x = A_q
    x = x + _A_ref(_layernorm(x, axis=-1), A_k, A_v, A_shift_k, A_ssm_k, A_ssm_D)
    x = x + _B_ref(_layernorm(x, axis=-1), B_wqkv, B_wo)
    x = x + _A_ref(_layernorm(x, axis=-1), A_k, A_v, A_shift_k, A_ssm_k, A_ssm_D)
    x = x + _B_ref(_layernorm(x, axis=-1), B_wqkv, B_wo)
    return x
```

```python
import functools
import numpy as np
import jax
import jax.numpy as jnp
from jax import lax
import jax.experimental.pallas as pl
import jax.experimental.pallas.tpu as pltpu

S, D = 2048, 512
NB = 4
BLK = S // NB
NFFT = 2 * BLK
N2 = BLK // 128
H, DH = 32, 16
TS = 512
NT_ = S // TS
f32 = jnp.float32
bf16 = jnp.bfloat16
NT = (((1,), (1,)), ((), ()))
SCOPES = False


class _noscope:
    def __enter__(self):
        return self

    def __exit__(self, *a):
        return False


def scope(name):
    return jax.named_scope(name) if SCOPES else _noscope()


def _dft_tables():
    k1 = np.concatenate([np.arange(0, 128, 2), np.arange(1, 128, 2)])
    n1 = np.arange(128)
    Fs = []
    for n2 in range(N2):
        th = 2 * np.pi * np.outer(k1 + 0.5, N2 * n1 + n2) / NFFT
        c = np.cos(th).reshape(16, 8, 128)
        s = -np.sin(th).reshape(16, 8, 128)
        Fs.append(np.concatenate([c, s], axis=1).reshape(256, 128))
    F = np.stack(Fs).astype(np.float32)
    FT = np.transpose(F, (0, 2, 1)) * (2.0 / NFFT)
    return F, FT


def _ln(x):
    m = jnp.mean(x, axis=-1, keepdims=True)
    xc = x - m
    v = jnp.mean(xc * xc, axis=-1, keepdims=True)
    return xc * lax.rsqrt(v + 1e-5)


def _phi(t):
    return jnp.where(t > 0, t + 1.0, jnp.exp(t)) + 1e-6


def _fft4(T, inverse):
    (ar, ai), (br, bi), (cr, ci), (dr, di) = T
    s0r, s0i = ar + cr, ai + ci
    d0r, d0i = ar - cr, ai - ci
    s1r, s1i = br + dr, bi + di
    d1r, d1i = br - dr, bi - di
    X0 = (s0r + s1r, s0i + s1i)
    X2 = (s0r - s1r, s0i - s1i)
    Xm = (d0r + d1i, d0i - d1r)
    Xp = (d0r - d1i, d0i + d1r)
    if inverse:
        return [X0, Xp, X2, Xm]
    return [X0, Xm, X2, Xp]


def _cat(ref, rows):
    return jnp.concatenate([ref[c, rows, :] for c in range(4)], axis=1)


def kernel(q_hbm, k_hbm, v_hbm, sk_hbm, h_hbm, dv_hbm, wqkv_hbm, wo_hbm, F_hbm, FT_hbm,
           o_hbm,
           q_v, k_v, v_v, sk_v, h_v, dv_v, wqkv_v, wo_v, F_v, FT_v, o_v,
           kf, vf, hT, ub, Tu, Th, Zb, y_s, x_s, pq_s, P_s, z_s, M_s, Mf, wT, wqT, wkT,
           sems, osems):
    copies = {}

    def add(name, src, dst):
        cp = pltpu.make_async_copy(src, dst, sems.at[len(copies)])
        copies[name] = cp
        cp.start()

    add("sk", sk_hbm, sk_v)
    add("dv", dv_hbm, dv_v)
    add("F", F_hbm, F_v)
    for i in range(NB):
        rs = pl.ds(i * BLK, BLK)
        add(f"k{i}", k_hbm.at[rs], k_v.at[rs])
        add(f"v{i}", v_hbm.at[rs], v_v.at[rs])
        add(f"h{i}", h_hbm.at[:, rs], h_v.at[:, rs])
    add("FT", FT_hbm, FT_v)
    add("wqkv", wqkv_hbm, wqkv_v)
    for i in range(NB):
        rs = pl.ds(i * BLK, BLK)
        add(f"q{i}", q_hbm.at[rs], q_v.at[rs])
    add("wo", wo_hbm, wo_v)

    for c in range(4):
        kf[c, 0:8, :] = jnp.zeros((8, 128), f32)
    copies["sk"].wait()
    copies["dv"].wait()
    copies["F"].wait()
    skT = sk_v[...].astype(f32)
    w = [skT[j:j + 1, :] for j in range(4)]

    def sld(ref, start):
        return jnp.concatenate(
            [ref[c, pl.ds(start, 128, stride=N2), :] for c in range(4)], axis=1)

    for i in range(NB):
        base = i * BLK
        with scope("prep_kv"):
            copies[f"k{i}"].wait()
            copies[f"v{i}"].wait()
            for c in range(4):
                ls = slice(c * 128, (c + 1) * 128)
                kf[c, 8 + base:8 + base + BLK, :] = k_v[base:base + BLK, ls].astype(f32)
                vf[c, base:base + BLK, :] = v_v[base:base + BLK, ls].astype(f32)
        with scope("fwd_u"):
            Ks = {}
            for o in range(-3, 4):
                Ks[o] = sld(kf, base + 8 + o)
            for n2 in range(N2):
                ks = Ks[n2] * w[0] + Ks[n2 - 1] * w[1] + Ks[n2 - 2] * w[2] + Ks[n2 - 3] * w[3]
                ks = ks.astype(bf16).astype(f32)
                u = (ks * sld(vf, base + n2)).astype(bf16)
                ub[i * N2 + n2] = u
                Tu[i * N2 + n2] = jnp.dot(F_v[n2], u, preferred_element_type=f32)
        with scope("prep_h"):
            copies[f"h{i}"].wait()
            for c in range(4):
                ls = slice(c * 128, (c + 1) * 128)
                hT[c, base:base + BLK, :] = h_v[ls, base:base + BLK].astype(f32).T
        with scope("fwd_h"):
            for n2 in range(N2):
                hh = sld(hT, base + n2).astype(bf16)
                Th[i * N2 + n2] = jnp.dot(F_v[n2], hh, preferred_element_type=f32)

    def mid(g, sign):
        r0 = pl.multiple_of(g * 16, 16)
        for c in range(D // 128):
            ls = slice(c * 128, (c + 1) * 128)

            def ld(ref, s):
                t = ref[s, pl.ds(r0, 16), ls]
                return (t[0:8], t[8:16])
            U = [_fft4([ld(Tu, i * N2 + n2) for n2 in range(N2)], False) for i in range(NB)]
            Hh = [_fft4([ld(Th, i * N2 + n2) for n2 in range(N2)], False) for i in range(NB)]
            G = [Hh[0]]
            for m in range(1, NB):
                if sign > 0:
                    G.append([(Hh[m][k2][0] - Hh[m - 1][k2][1], Hh[m][k2][1] + Hh[m - 1][k2][0])
                              for k2 in range(N2)])
                else:
                    G.append([(Hh[m][k2][0] + Hh[m - 1][k2][1], Hh[m][k2][1] - Hh[m - 1][k2][0])
                              for k2 in range(N2)])
            for j in range(NB):
                C = []
                for k2 in range(N2):
                    cr = ci = None
                    for i in range(j + 1):
                        (ur, ui), (gr, gi) = U[i][k2], G[j - i][k2]
                        pr = ur * gr - ui * gi
                        pi = ur * gi + ui * gr
                        cr = pr if cr is None else cr + pr
                        ci = pi if ci is None else ci + pi
                    C.append((cr, ci))
                Z = _fft4(C, True)
                for n2 in range(N2):
                    Zb[j * N2 + n2, pl.ds(r0, 16), ls] = jnp.concatenate(
                        [Z[n2][0], Z[n2][1]], axis=0).astype(bf16)

    with scope("mid"):
        lax.fori_loop(0, 8, lambda g, c: (mid(g, 1), c)[1], 0)
        lax.fori_loop(8, 16, lambda g, c: (mid(g, -1), c)[1], 0)

    dv4 = dv_v[...].astype(f32)
    dv = jnp.concatenate([dv4[c:c + 1, :] for c in range(4)], axis=1)
    copies["FT"].wait()

    def inv_block(j, carry):
        base = pl.multiple_of(j * BLK, BLK)
        for n2 in range(N2):
            yy = jnp.dot(FT_v[n2], Zb[j * N2 + n2], preferred_element_type=f32)
            yy = yy + ub[j * N2 + n2].astype(f32) * dv
            for c in range(4):
                y_s[c, pl.ds(base + n2, 128, stride=N2), :] = yy[:, c * 128:(c + 1) * 128]
        return carry

    with scope("inv"):
        lax.fori_loop(0, NB, inv_block, 0)

    with scope("wprep"):
        copies["wqkv"].wait()
        for which, dst in ((0, wqT), (1, wkT)):
            for c in range(4):
                wT[c] = wqkv_v[c * 128:(c + 1) * 128, which * D:(which + 1) * D].astype(f32).T
            for dh in range(DH):
                blk = jnp.concatenate(
                    [wT[c, pl.ds(dh, H, stride=DH), :] for c in range(4)], axis=1)
                dst[dh * H:(dh + 1) * H, :] = blk.astype(bf16)

    row = lax.broadcasted_iota(jnp.int32, (128, 128), 0) % 8
    col = lax.broadcasted_iota(jnp.int32, (128, 128), 1) // DH
    mask = row == col

    def phase_a(x, rows):
        xn = _ln(x).astype(bf16)
        qq = lax.dot_general(xn, wqT[...], NT, preferred_element_type=f32)
        pq_s[rows, :] = _phi(qq)
        kT = lax.dot_general(wkT[...], xn, NT, preferred_element_type=f32)
        pkT = _phi(kT)
        zz = pkT[:, 0:128]
        for c in range(1, TS // 128):
            zz = zz + pkT[:, c * 128:(c + 1) * 128]
        z_s[...] += zz
        P_s[...] += jnp.dot(pkT.astype(bf16), xn, preferred_element_type=f32)

    def mid_b():
        for j in range(4):
            Pj = jnp.concatenate(
                [P_s[dh * H + 8 * j: dh * H + 8 * j + 8, :] for dh in range(DH)], axis=0)
            kv = jnp.dot(Pj.astype(bf16), wqkv_v[:, 2 * D + 128 * j:2 * D + 128 * (j + 1)],
                         preferred_element_type=f32)
            kv = jnp.where(mask, kv, 0.0).astype(bf16)
            Mj = jnp.dot(kv, wo_v[128 * j:128 * (j + 1), :], preferred_element_type=f32)
            for dh in range(DH):
                Mf[dh * H + 8 * j: dh * H + 8 * j + 8, :] = Mj[8 * dh:8 * dh + 8, :]
        M_s[...] = Mf[...].astype(bf16)
        return jnp.sum(z_s[...].T, axis=0, keepdims=True)

    def phase_b(rows, z):
        pq = pq_s[rows, :]
        t = pq * z
        t = (t[:, 0:128] + t[:, 128:256]) + (t[:, 256:384] + t[:, 384:512])
        t = t + pltpu.roll(t, 32, 1)
        t = t + pltpu.roll(t, 64, 1)
        r = 1.0 / (t + 1e-6)
        pqn = (pq * jnp.concatenate([r, r, r, r], axis=1)).astype(bf16)
        return jnp.dot(pqn, M_s[...], preferred_element_type=f32)

    def reset():
        P_s[...] = jnp.zeros_like(P_s)
        z_s[...] = jnp.zeros_like(z_s)

    reset()
    for i in range(NB):
        copies[f"q{i}"].wait()

    def loop1(t, carry):
        rows = pl.ds(pl.multiple_of(t * TS, TS), TS)
        x = q_v[rows, :].astype(f32)
        x = x + _ln(x) * _cat(y_s, rows)
        x_s[rows, :] = x
        phase_a(x, rows)
        return carry

    with scope("loop1"):
        lax.fori_loop(0, NT_, loop1, 0, unroll=True)
    copies["wo"].wait()
    with scope("mid_b"):
        z1 = mid_b()
        reset()

    def loop2(t, carry):
        rows = pl.ds(pl.multiple_of(t * TS, TS), TS)
        x = x_s[rows, :] + phase_b(rows, z1)
        x = x + _ln(x) * _cat(y_s, rows)
        x_s[rows, :] = x
        phase_a(x, rows)
        return carry

    with scope("loop2"):
        lax.fori_loop(0, NT_, loop2, 0, unroll=True)
    with scope("mid_b"):
        z2 = mid_b()

    def out_copy(t):
        rows = pl.ds(pl.multiple_of(t * TS, TS), TS)
        return pltpu.make_async_copy(o_v.at[rows], o_hbm.at[rows], osems.at[t])

    def loop3(t, carry):
        rows = pl.ds(pl.multiple_of(t * TS, TS), TS)
        x = x_s[rows, :] + phase_b(rows, z2)
        o_v[rows, :] = x.astype(bf16)
        out_copy(t).start()
        return carry

    with scope("loop3"):
        lax.fori_loop(0, NT_, loop3, 0, unroll=True)
        for t in range(NT_):
            out_copy(t).wait()


@jax.jit
def pallas_interleave_layers__ssm_conv_h3__linear_attn_block__prompt_kernel(
        A_q, A_k, A_v, A_shift_k, A_ssm_k, A_ssm_D, B_x, B_wqkv, B_wo):
    F, FT = _dft_tables()
    F = jnp.asarray(F, dtype=bf16)
    FT = jnp.asarray(FT, dtype=bf16)
    q = A_q.reshape(S, D)
    k = A_k.reshape(S, D)
    v = A_v.reshape(S, D)
    dv = A_ssm_D.reshape(4, 128)
    anyspec = pl.BlockSpec(memory_space=pl.ANY)
    out = pl.pallas_call(
        kernel,
        out_shape=jax.ShapeDtypeStruct((S, D), bf16),
        in_specs=[anyspec] * 10,
        out_specs=anyspec,
        scratch_shapes=[
            pltpu.VMEM((S, D), bf16),
            pltpu.VMEM((S, D), bf16),
            pltpu.VMEM((S, D), bf16),
            pltpu.VMEM((4, D), bf16),
            pltpu.VMEM((D, S), bf16),
            pltpu.VMEM((4, 128), bf16),
            pltpu.VMEM((D, 3 * D), bf16),
            pltpu.VMEM((D, D), bf16),
            pltpu.VMEM((N2, 256, 128), bf16),
            pltpu.VMEM((N2, 128, 256), bf16),
            pltpu.VMEM((S, D), bf16),
            pltpu.VMEM((4, S + 8, 128), f32),
            pltpu.VMEM((4, S, 128), f32),
            pltpu.VMEM((4, S, 128), f32),
            pltpu.VMEM((16, 128, D), bf16),
            pltpu.VMEM((16, 256, D), f32),
            pltpu.VMEM((16, 256, D), f32),
            pltpu.VMEM((16, 256, D), bf16),
            pltpu.VMEM((4, S, 128), f32),
            pltpu.VMEM((S, D), f32),
            pltpu.VMEM((S, D), f32),
            pltpu.VMEM((D, D), f32),
            pltpu.VMEM((D, 128), f32),
            pltpu.VMEM((D, D), bf16),
            pltpu.VMEM((D, D), f32),
            pltpu.VMEM((4, D, 128), f32),
            pltpu.VMEM((D, D), bf16),
            pltpu.VMEM((D, D), bf16),
            pltpu.SemaphoreType.DMA((24,)),
            pltpu.SemaphoreType.DMA((NT_,)),
        ],
        compiler_params=pltpu.CompilerParams(vmem_limit_bytes=110 * 1024 * 1024),
    )(q, k, v, A_shift_k.T, A_ssm_k, dv, B_wqkv, B_wo, F, FT)
    return out.reshape(1, S, D)
```

```python
import os
import numpy as np
import jax
import jax.numpy as jnp
from jax import lax
import jax.experimental.pallas as pl
import jax.experimental.pallas.tpu as pltpu

S, D = 2048, 512
NB = 4
BLK = S // NB
NFFT = 2 * BLK
N2 = BLK // 128
H, DH = 32, 16
TS = 512
NT_ = S // TS
f32 = jnp.float32
bf16 = jnp.bfloat16
u32 = jnp.uint32
NT = (((1,), (1,)), ((), ()))
SCOPES = False

SCHED = [
    ("A0", "k00 v00 h00", "H00 U00"),
    ("A1", "k01 v01 h01", "H01 a00 U01 b00"),
    ("A2", "k02 v02 h02 k03 v03 h03", "H02 a01 U02 H03 b01 U03"),
    ("A3", "wk", "wk a02 b02 a03 b03"),
    ("K0", "q0 wq", "wq L0 K00 K01 K02 K03"),
    ("F1", "k1 v1 h1", "P00 U10 H10 U11 H11 P01 U12 H12 U13 H13"),
    ("C0", "k2 v2 h2", "Q00 a10 H20 b10 P02 U20 a11 H21 b11 Q01 U21 a12 H22 b12 P03 U22 a13 H23 b13"),
    ("K1", "q1", "L1 Q02 K10 Q03 K11 U23 K12 K13"),
    ("C1", "k3 v3 h3",
     "P10 a20 H30 b20 Q10 U30 a21 P11 b21 H31 U31 P12 a22 H32 b22 Q11 U32 a23 P13 b23 H33 U33"),
    ("K2", "q2", "L2 Q12 K20 Q13 K21 K22 K23"),
    ("C2", "", "P20 a30 Q20 b30 P21 a31 Q21 b31 P22 a32 Q22 b32 P23 a33 b33"),
    ("K3", "q3 wv wo", "L3 Q23 K30 K31 K32 K33"),
]
LAST = NT_ - 1
DEFER = int(os.environ.get('DEFER', '0'))
XORD = os.environ.get('XORD', 'P0 P1 P2 P3 Q0 Q1 Q2 Q3')
ZEARLY = int(os.environ.get('ZEARLY', '0'))
STG = int(os.environ.get('STG', '3'))
Y0ORD = os.environ.get('Y0ORD', 'O0 O1 K0 O2 K1 K2 K3 O3')


class _noscope:
    def __enter__(self):
        return self

    def __exit__(self, *a):
        return False


def scope(name):
    return jax.named_scope(name) if SCOPES else _noscope()


def _dft_tables():
    shape = (256, 128)
    r = lax.broadcasted_iota(jnp.int32, shape, 0)
    n1 = lax.broadcasted_iota(jnp.int32, shape, 1)
    i = ((r >> 4) << 3) + (r & 7)
    a = jnp.where(i < 64, 4 * i + 1, 4 * i - 253)
    m0 = a * (N2 * n1) + ((r & 8) << 6)
    out = []
    for n2 in range(N2):
        m = (m0 + n2 * a) & 2047
        x = (512 - jnp.minimum(m, 2048 - m)).astype(f32) * (np.pi / 1024)
        x2 = x * x
        c = [0.9999999765893761, -0.1666664763431631, 0.008332899817899943,
             -0.00019800897428633393, 2.5904878274341777e-06]
        acc = c[4]
        for k in (3, 2, 1, 0):
            acc = acc * x2 + c[k]
        out.append(x * acc)
    return out


def _ln(x):
    m = jnp.mean(x, axis=-1, keepdims=True)
    xc = x - m
    v = jnp.mean(xc * xc, axis=-1, keepdims=True)
    return xc * lax.rsqrt(v + 1e-5)


def _phi(t):
    return jnp.where(t > 0, t + 1.0, jnp.exp(t)) + 1e-6


def _fft4(T, inverse):
    (ar, ai), (br, bi), (cr, ci), (dr, di) = T
    s0r, s0i = ar + cr, ai + ci
    d0r, d0i = ar - cr, ai - ci
    s1r, s1i = br + dr, bi + di
    d1r, d1i = br - dr, bi - di
    X0 = (s0r + s1r, s0i + s1i)
    X2 = (s0r - s1r, s0i - s1i)
    Xm = (d0r + d1i, d0i - d1r)
    Xp = (d0r - d1i, d0i + d1r)
    if inverse:
        return [X0, Xp, X2, Xm]
    return [X0, Xm, X2, Xp]


def _pk(x):
    return pltpu.bitcast(x, u32)


def _upk(x):
    return pltpu.bitcast(x, bf16)


def _ds(t, scale, off, size):
    if isinstance(t, int):
        return pl.ds(t * scale + off, size)
    return pl.ds(pl.multiple_of(t * scale + off, size), size)


def _cat(ref, rows):
    return jnp.concatenate([ref[c, rows, :] for c in range(4)], axis=1)


def _catp(ref, rows=slice(None)):
    return jnp.concatenate([_upk(ref[c, rows, :]) for c in range(4)], axis=1)


def kernel(q_hbm, k_hbm, v_hbm, sk_hbm, h_hbm, dv_hbm, wqkv_hbm, wo_hbm,
           o_hbm,
           q_v, k_v, v_v, sk_v, h_v, dv_v, wqkv_v, wo_v, o_v,
           F_v, FT_v, kf, vf, hT, Us, Hs, y_s, ya_s, x_s, xn_s, pk_s, pq_s, P_s, z_s, zr_s,
           M_s, Mf, wqT, wkT, cw, pn_s,
           sems, osems, bsem):
    copies = {}

    def add(name, src, dst):
        cp = pltpu.make_async_copy(src, dst, sems.at[len(copies)])
        copies[name] = cp
        cp.start()

    def add_kvh(i):
        rs = pl.ds(i * BLK, BLK)
        add(f"k{i}", k_hbm.at[rs], k_v.at[rs])
        add(f"v{i}", v_hbm.at[rs], v_v.at[rs])
        add(f"h{i}", h_hbm.at[:, rs], h_v.at[:, rs])

    def add_q(i):
        rs = pl.ds(i * BLK, BLK)
        add(f"q{i}", q_hbm.at[rs], q_v.at[rs])

    def add_w(name, j):
        cs = pl.ds(j * D, D)
        add(name, wqkv_hbm.at[:, cs], wqkv_v.at[:, cs])

    add("sk", sk_hbm, sk_v)
    add("dv", dv_hbm, dv_v)
    for c in range(4):
        rs, ls = pl.ds(0, BLK), pl.ds(c * 128, 128)
        add(f"k0{c}", k_hbm.at[rs, ls], k_v.at[rs, ls])
        add(f"v0{c}", v_hbm.at[rs, ls], v_v.at[rs, ls])
        add(f"h0{c}", h_hbm.at[ls, rs], h_v.at[ls, rs])
    add_w("wk", 1)
    add_q(0)
    add_w("wq", 0)
    add_kvh(1)
    add_kvh(2)
    add_q(1)
    add_kvh(3)
    add_q(2)
    add_q(3)
    add_w("wv", 2)
    add("wo", wo_hbm, wo_v)

    def wait(*names):
        for n in names:
            copies[n].wait()

    def barrier():
        pl.semaphore_signal(bsem, 1)
        pl.semaphore_wait(bsem, 1)

    for n2, tab in enumerate(_dft_tables()):
        F_v[n2] = _pk(tab.astype(bf16))
        for hf in range(2):
            ft = (tab[128 * hf:128 * (hf + 1), :] * (2.0 / NFFT)).T
            FT_v[n2, hf] = _pk(ft.astype(bf16))

    for c in range(4):
        kf[c, 0:8, :] = jnp.zeros((8, 128), f32)
    wait("sk", "dv")
    skT = sk_v[...].astype(f32)
    dv4 = dv_v[...].astype(f32)
    for c in range(4):
        cw[c, 0:4, :] = skT[:, c * 128:(c + 1) * 128]
        cw[c, 4:5, :] = dv4[c:c + 1, :]

    def split(T, g):
        return (T[16 * g:16 * g + 8], T[16 * g + 8:16 * g + 16])

    def join(val):
        return jnp.concatenate([val[0], val[1]], axis=0)

    def FU(i, c):
        base = i * BLK
        ls = pl.ds(c * 128, 128)
        kf[c, pl.ds(8 + base, BLK), :] = k_v[pl.ds(base, BLK), ls].astype(f32)
        vf[c, pl.ds(base, BLK), :] = v_v[pl.ds(base, BLK), ls].astype(f32)
        Ks = {o: kf[c, pl.ds(base + 8 + o, 128, stride=N2), :] for o in range(-3, 4)}
        wc = [cw[c, j:j + 1, :] for j in range(4)]
        T = []
        for n2 in range(N2):
            ks = (Ks[n2] * wc[0] + Ks[n2 - 1] * wc[1]) + (Ks[n2 - 2] * wc[2] + Ks[n2 - 3] * wc[3])
            u = (ks * vf[c, pl.ds(base + n2, 128, stride=N2), :]).astype(bf16)
            T.append(jnp.dot(_upk(F_v[n2]), u, preferred_element_type=f32))
        for g in range(16):
            U = _fft4([split(T[n2], g) for n2 in range(N2)], False)
            for k2 in range(N2):
                Us[c, i * N2 + k2, 16 * g:16 * g + 16, :] = join(U[k2])

    def FH(i, c):
        base = i * BLK
        hT[c, pl.ds(base, BLK), :] = h_v[pl.ds(c * 128, 128), pl.ds(base, BLK)].astype(f32).T
        T = []
        for n2 in range(N2):
            hh = hT[c, pl.ds(base + n2, 128, stride=N2), :].astype(bf16)
            T.append(jnp.dot(_upk(F_v[n2]), hh, preferred_element_type=f32))
        for g in range(16):
            Hj = _fft4([split(T[n2], g) for n2 in range(N2)], False)
            if i == 0:
                Hj = [(re + cw[c, 4:5, :], im) for re, im in Hj]
            for k2 in range(N2):
                Hs[c, i * N2 + k2, 16 * g:16 * g + 16, :] = join(Hj[k2])

    def INV(j, c, half):
        Zs = [[] for _ in range(N2)]
        for g in range(8 * half, 8 * half + 8):
            def ld(ref, s):
                t = ref[c, s, 16 * g:16 * g + 16, :]
                return (t[0:8], t[8:16])
            C = []
            for k2 in range(N2):
                Hm = [ld(Hs, m * N2 + k2) for m in range(j + 1)]
                cr = ci = None
                for m in range(j + 1):
                    gr, gi = Hm[m]
                    if m > 0:
                        pr_, pi_ = Hm[m - 1]
                        if half == 0:
                            gr, gi = gr - pi_, gi + pr_
                        else:
                            gr, gi = gr + pi_, gi - pr_
                    ur, ui = ld(Us, (j - m) * N2 + k2)
                    pr = ur * gr - ui * gi
                    pi = ur * gi + ui * gr
                    cr = pr if cr is None else cr + pr
                    ci = pi if ci is None else ci + pi
                C.append((cr, ci))
            Z = _fft4(C, True)
            for n2 in range(N2):
                Zs[n2].append(join(Z[n2]).astype(bf16))
        dst = ya_s if half == 0 else y_s
        for n2 in range(N2):
            dst[c, pl.ds(j * BLK + n2, 128, stride=N2), :] = jnp.dot(
                _upk(FT_v[n2, half]), jnp.concatenate(Zs[n2], axis=0), preferred_element_type=f32)

    def wprep(which, dst):
        pr = lax.broadcasted_iota(jnp.int32, (128, 128), 0)
        pc = lax.broadcasted_iota(jnp.int32, (128, 128), 1)
        perm = jnp.where(pc == (pr % 8) * DH + pr // 8, 1.0, 0.0).astype(bf16)
        outs = []
        for a in range(4):
            wa = wqkv_v[:, which * D + 128 * a:which * D + 128 * (a + 1)]
            outs.append(lax.dot_general(perm, wa, NT, preferred_element_type=f32))
        for dh in range(DH):
            blk = jnp.concatenate([outs[a][8 * dh:8 * dh + 8, :] for a in range(4)], axis=0)
            blk = blk.astype(bf16)
            for c in range(4):
                dst[c, dh * H // 2:(dh + 1) * H // 2, :] = _pk(blk[:, c * 128:(c + 1) * 128])

    def a_layer(src, t, slot=None):
        slot = t if slot is None else slot
        rows = _ds(t, TS, 0, TS)
        x = src[rows, :].astype(f32)
        x = x + _ln(x) * (_cat(y_s, rows) + _cat(ya_s, rows))
        x_s[rows, :] = x
        xn = _ln(x).astype(bf16)
        for c in range(4):
            xn_s[c, pl.ds(slot * (TS // 2), TS // 2), :] = _pk(xn[:, c * 128:(c + 1) * 128])

    def KT(t, c, slot=None):
        slot = t if slot is None else slot
        xn = _catp(xn_s, pl.ds(slot * (TS // 2) + c * 64, 64))
        kT = lax.dot_general(_catp(wkT), xn, NT, preferred_element_type=f32)
        pkT = _phi(kT)
        if isinstance(t, int) and t == 0 and c == 0:
            z_s[...] = pkT
        else:
            z_s[...] += pkT
        pk_s[c] = _pk(pkT.astype(bf16))

    def PP(t, c, slot=None):
        slot = t if slot is None else slot
        pp = jnp.dot(_catp(pk_s), _upk(xn_s[c, pl.ds(slot * (TS // 2), TS // 2), :]),
                     preferred_element_type=f32)
        if isinstance(t, int) and t == 0:
            P_s[c] = pp
        else:
            P_s[c] += pp

    def QQ(t, c, slot=None):
        slot = t if slot is None else slot
        qq = lax.dot_general(
            _catp(xn_s, pl.ds(slot * (TS // 2), TS // 2)), _catp(wqT, pl.ds(c * 64, 64)), NT,
            preferred_element_type=f32)
        pq_s[c, _ds(t, TS, 0, TS), :] = qq if DEFER else _phi(qq)

    def mid_b():
        row = lax.broadcasted_iota(jnp.int32, (128, 128), 0) % 8
        col = lax.broadcasted_iota(jnp.int32, (128, 128), 1) // DH
        mask = row == col
        for j in range(4):
            Pj = jnp.concatenate(
                [_cat(P_s, pl.ds(dh * H + 8 * j, 8)) for dh in range(DH)], axis=0)
            kv = jnp.dot(Pj.astype(bf16), wqkv_v[:, 2 * D + 128 * j:2 * D + 128 * (j + 1)],
                         preferred_element_type=f32)
            kv = jnp.where(mask, kv, 0.0).astype(bf16)
            Mj = jnp.dot(kv, wo_v[128 * j:128 * (j + 1), :], preferred_element_type=f32)
            for dh in range(DH):
                Mf[dh * H + 8 * j: dh * H + 8 * j + 8, :] = Mj[8 * dh:8 * dh + 8, :]
        for c in range(4):
            M_s[c] = _pk(Mf[:, c * 128:(c + 1) * 128].astype(bf16))

    def zrow():
        zr_s[...] = jnp.sum(z_s[...].T, axis=0, keepdims=True)

    def PQN(r0, n):
        rows = pl.ds(r0, n)
        z = zr_s[...]
        pq = [_phi(pq_s[c, rows, :]) if DEFER else pq_s[c, rows, :] for c in range(4)]
        tt = [pq[c] * z[:, c * 128:(c + 1) * 128] for c in range(4)]
        tt = (tt[0] + tt[1]) + (tt[2] + tt[3])
        tt = tt + pltpu.roll(tt, 32, 1)
        tt = tt + pltpu.roll(tt, 64, 1)
        r = 1.0 / (tt + 1e-6)
        return [(pq[c] * r).astype(bf16) for c in range(4)]

    def OUT(r0, n, pqn=None):
        if pqn is None:
            pqn = _catp(pn_s, pl.ds((r0 - STG * TS) // 2, n // 2))
        else:
            pqn = jnp.concatenate(pqn, axis=1)
        return x_s[pl.ds(r0, n), :] + jnp.dot(pqn, _catp(M_s), preferred_element_type=f32)

    xtiles = [t for t in range(NT_) if t != STG]
    pieces = [(t * TS, TS) for t in xtiles] + [
        (STG * TS, 256), (STG * TS + 256, 128), (STG * TS + 384, 128)]

    def out_copy(i):
        rows = pl.ds(*pieces[i])
        return pltpu.make_async_copy(o_v.at[rows], o_hbm.at[rows], osems.at[i])

    ops = {"H": FH, "U": FU, "a": lambda j, c: INV(j, c, 0), "b": lambda j, c: INV(j, c, 1),
           "K": KT, "P": PP, "Q": QQ}
    for name, waits, toks in SCHED:
        with scope(name):
            if waits:
                wait(*waits.split())
            else:
                barrier()
            for tok in toks.split():
                if tok == "wk":
                    wprep(1, wkT)
                elif tok == "wq":
                    wprep(0, wqT)
                elif tok[0] == "L":
                    a_layer(q_v, int(tok[1]))
                else:
                    ops[tok[0]](int(tok[1]), int(tok[2]))

    def layer(l, carry):
        with scope("X"):
            for tok in XORD.split():
                if tok == "|":
                    barrier()
                elif tok == "z":
                    zrow()
                else:
                    ops[tok[0]](LAST, int(tok[1]))
            mid_b()
            if "z" not in XORD:
                zrow()
            P_s[...] = jnp.zeros_like(P_s)
            pl3 = PQN(STG * TS, TS)
            for c in range(4):
                pn_s[c] = _pk(pl3[c])
            for i, t in enumerate(xtiles):
                res = OUT(t * TS, TS, PQN(t * TS, TS))
                x_s[pl.ds(t * TS, TS), :] = res
                o_v[pl.ds(t * TS, TS), :] = res.astype(bf16)
                out_copy(i).start()

        @pl.when(l == 0)
        def _():
            with scope("Y0"):
                a_layer(x_s, 0, LAST)
                for tok in Y0ORD.split():
                    c = int(tok[1])
                    if tok[0] == "O":
                        r0 = STG * TS + c * 128
                        x_s[pl.ds(r0, 128), :] = OUT(r0, 128)
                    else:
                        KT(0, c, LAST)
                for t in range(NT_ - 1):
                    out_copy(t).wait()

            def ybody(t, carry2):
                for c in range(4):
                    PP(t - 1, c, LAST)
                for c in range(4):
                    QQ(t - 1, c, LAST)
                a_layer(x_s, t, LAST)
                for c in range(4):
                    KT(t, c, LAST)
                return carry2
            with scope("Y1"):
                lax.fori_loop(1, NT_, ybody, 0)
        return carry

    lax.fori_loop(0, 2, layer, 0)

    with scope("Z"):
        for i in range(NT_ - 1, len(pieces)):
            r0, n = pieces[i]
            o_v[pl.ds(r0, n), :] = OUT(r0, n).astype(bf16)
            out_copy(i).start()
        for i in range(len(pieces)):
            out_copy(i).wait()


@jax.jit
def pallas_interleave_layers__ssm_conv_h3__linear_attn_block__prompt_kernel(
        A_q, A_k, A_v, A_shift_k, A_ssm_k, A_ssm_D, B_x, B_wqkv, B_wo):
    anyspec = pl.BlockSpec(memory_space=pl.ANY)
    out = pl.pallas_call(
        kernel,
        out_shape=jax.ShapeDtypeStruct((S, D), bf16),
        in_specs=[anyspec] * 8,
        out_specs=anyspec,
        scratch_shapes=[
            pltpu.VMEM((S, D), bf16),
            pltpu.VMEM((S, D), bf16),
            pltpu.VMEM((S, D), bf16),
            pltpu.VMEM((4, D), bf16),
            pltpu.VMEM((D, S), bf16),
            pltpu.VMEM((4, 128), bf16),
            pltpu.VMEM((D, 3 * D), bf16),
            pltpu.VMEM((D, D), bf16),
            pltpu.VMEM((S, D), bf16),
            pltpu.VMEM((N2, 128, 128), u32),
            pltpu.VMEM((N2, 2, 64, 128), u32),
            pltpu.VMEM((4, S + 8, 128), f32),
            pltpu.VMEM((4, S, 128), f32),
            pltpu.VMEM((4, S, 128), f32),
            pltpu.VMEM((4, 16, 256, 128), f32),
            pltpu.VMEM((4, 16, 256, 128), f32),
            pltpu.VMEM((4, S, 128), f32),
            pltpu.VMEM((4, S, 128), f32),
            pltpu.VMEM((S, D), f32),
            pltpu.VMEM((4, S // 2, 128), u32),
            pltpu.VMEM((4, D // 2, 128), u32),
            pltpu.VMEM((4, S, 128), f32),
            pltpu.VMEM((4, D, 128), f32),
            pltpu.VMEM((D, 128), f32),
            pltpu.VMEM((1, D), f32),
            pltpu.VMEM((4, D // 2, 128), u32),
            pltpu.VMEM((D, D), f32),
            pltpu.VMEM((4, D // 2, 128), u32),
            pltpu.VMEM((4, D // 2, 128), u32),
            pltpu.VMEM((4, 8, 128), f32),
            pltpu.VMEM((4, TS // 2, 128), u32),
            pltpu.SemaphoreType.DMA((32,)),
            pltpu.SemaphoreType.DMA((8,)),
            pltpu.SemaphoreType.REGULAR,
        ],
        compiler_params=pltpu.CompilerParams(vmem_limit_bytes=110 * 1024 * 1024),
    )(A_q.reshape(S, D), A_k.reshape(S, D), A_v.reshape(S, D), A_shift_k.T, A_ssm_k,
      A_ssm_D.reshape(4, 128), B_wqkv, B_wo)
    return out.reshape(1, S, D)
```

```python
import numpy as np
import jax
import jax.numpy as jnp
from jax import lax
import jax.experimental.pallas as pl
import jax.experimental.pallas.tpu as pltpu

S, D = 2048, 512
NB = 4
BLK = S // NB
NFFT = 2 * BLK
N2 = BLK // 128
H, DH = 32, 16
TS = 512
NT_ = S // TS
f32 = jnp.float32
bf16 = jnp.bfloat16
u32 = jnp.uint32
NT = (((1,), (1,)), ((), ()))

SCHED = [
    ("A0", "k00 v00 h00", "U00 H00"),
    ("A1", "k01 v01 h01", "b00 a00 H01 U01"),
    ("A2", "k02 v02 h02 k03 v03 h03", "U03 a01 H02 b01 H03 U02"),
    ("A3", "wk", "wk a02 b02 a03 b03"),
    ("K0", "q0 wq", "wq L0 K00 K01 K02 K03"),
    ("F1", "k1 v1 h1", "P00 U10 U13 H10 P01 U12 U11 H11 H12 H13"),
    ("C0", "k2 v2 h2",
     "P02 a10 H20 b10 P03 a11 H21 U22 b11 Q00 a12 H22 b12 Q01 a13 H23 b13 U20 U21"),
    ("K1", "q1 k3 v3 h3", "L1 Q02 Q03 K13 K12 K11 H33 K10 U23"),
    ("C1", "",
     "P10 a20 H30 b20 P11 a21 H31 b21 P12 a22 H32 b22 P13 a23 Q10 b23 U30 U31 U32 U33"),
    ("K2", "q2", "L2 Q12 Q13 K22 K23 K21 Q11 K20 a30"),
    ("C2", "", "P20 a33 Q20 b30 P21 a31 Q21 b31 P22 a32 Q22 b32 P23 b33"),
    ("K3", "q3 wv wo", "L3 Q23 K30 K31 K32 K33"),
]
LAST = NT_ - 1


def _dft_tables():
    shape = (256, 128)
    r = lax.broadcasted_iota(jnp.int32, shape, 0)
    n1 = lax.broadcasted_iota(jnp.int32, shape, 1)
    i = ((r >> 4) << 3) + (r & 7)
    a = jnp.where(i < 64, 4 * i + 1, 4 * i - 253)
    m0 = a * (N2 * n1) + ((r & 8) << 6)
    out = []
    for n2 in range(N2):
        m = (m0 + n2 * a) & 2047
        x = (512 - jnp.minimum(m, 2048 - m)).astype(f32) * (np.pi / 1024)
        x2 = x * x
        c = [0.9999999765893761, -0.1666664763431631, 0.008332899817899943,
             -0.00019800897428633393, 2.5904878274341777e-06]
        acc = c[4]
        for k in (3, 2, 1, 0):
            acc = acc * x2 + c[k]
        out.append(x * acc)
    return out


def _ln(x):
    m = jnp.mean(x, axis=-1, keepdims=True)
    xc = x - m
    v = jnp.mean(xc * xc, axis=-1, keepdims=True)
    return xc * lax.rsqrt(v + 1e-5)


def _phi(t):
    return jnp.where(t > 0, t + 1.0, jnp.exp(t)) + 1e-6


def _fft4(T, inverse):
    (ar, ai), (br, bi), (cr, ci), (dr, di) = T
    s0r, s0i = ar + cr, ai + ci
    d0r, d0i = ar - cr, ai - ci
    s1r, s1i = br + dr, bi + di
    d1r, d1i = br - dr, bi - di
    X0 = (s0r + s1r, s0i + s1i)
    X2 = (s0r - s1r, s0i - s1i)
    Xm = (d0r + d1i, d0i - d1r)
    Xp = (d0r - d1i, d0i + d1r)
    if inverse:
        return [X0, Xp, X2, Xm]
    return [X0, Xm, X2, Xp]


def _pk(x):
    return pltpu.bitcast(x, u32)


def _upk(x):
    return pltpu.bitcast(x, bf16)


def _ds(t, scale, off, size):
    if isinstance(t, int):
        return pl.ds(t * scale + off, size)
    return pl.ds(pl.multiple_of(t * scale + off, size), size)


def _cat(ref, rows):
    return jnp.concatenate([ref[c, rows, :] for c in range(4)], axis=1)


def _catp(ref, rows=pl.ds(0, D // 2)):
    return jnp.concatenate([_upk(ref[c, rows, :]) for c in range(4)], axis=1)


def kernel(q_hbm, k_hbm, v_hbm, sk_hbm, h_hbm, dv_hbm, wqkv_hbm, wo_hbm,
           o_hbm,
           q_v, k_v, v_v, sk_v, h_v, dv_v, wqkv_v, wo_v, o_v,
           F_v, FT_v, kf, vf, hT, Us, Hs, y_s, ya_s, x_s, xn_s, pk_s, pq_s, P_s, z_s, zr_s,
           M_s, wqT, wkT, cw, pn_s,
           sems, osems, bsem):
    copies = {}

    def add(name, src, dst):
        cp = pltpu.make_async_copy(src, dst, sems.at[len(copies)])
        copies[name] = cp
        cp.start()

    def add_kvh(i):
        rs = pl.ds(i * BLK, BLK)
        add(f"k{i}", k_hbm.at[rs], k_v.at[rs])
        add(f"v{i}", v_hbm.at[rs], v_v.at[rs])
        add(f"h{i}", h_hbm.at[:, rs], h_v.at[:, rs])

    def add_q(i):
        rs = pl.ds(i * BLK, BLK)
        add(f"q{i}", q_hbm.at[rs], q_v.at[rs])

    def add_w(name, j):
        cs = pl.ds(j * D, D)
        add(name, wqkv_hbm.at[:, cs], wqkv_v.at[:, cs])

    add("sk", sk_hbm, sk_v)
    add("dv", dv_hbm, dv_v)
    for c in range(4):
        rs, ls = pl.ds(0, BLK), pl.ds(c * 128, 128)
        add(f"k0{c}", k_hbm.at[rs, ls], k_v.at[rs, ls])
        add(f"v0{c}", v_hbm.at[rs, ls], v_v.at[rs, ls])
        add(f"h0{c}", h_hbm.at[ls, rs], h_v.at[ls, rs])
    add_w("wk", 1)
    add_q(0)
    add_w("wq", 0)
    add_kvh(1)
    add_kvh(2)
    add_q(1)
    add_kvh(3)
    add_q(2)
    add_q(3)
    add_w("wv", 2)
    add("wo", wo_hbm, wo_v)

    def wait(*names):
        for n in names:
            copies[n].wait()

    def barrier():
        pl.semaphore_signal(bsem, 1)
        pl.semaphore_wait(bsem, 1)

    for n2, tab in enumerate(_dft_tables()):
        F_v[n2] = _pk(tab.astype(bf16))
        for hf in range(2):
            ft = (tab[128 * hf:128 * (hf + 1), :] * (2.0 / NFFT)).T
            FT_v[n2, hf] = _pk(ft.astype(bf16))

    for c in range(4):
        kf[c, 0:8, :] = jnp.zeros((8, 128), u32)
    wait("sk", "dv")
    skT = sk_v[...].astype(f32)
    dv4 = dv_v[...].astype(f32)
    for c in range(4):
        cw[c, 0:4, :] = skT[:, c * 128:(c + 1) * 128]
        cw[c, 4:5, :] = dv4[c:c + 1, :]

    def split(T, g):
        return (T[16 * g:16 * g + 8], T[16 * g + 8:16 * g + 16])

    def join(val):
        return jnp.concatenate([val[0], val[1]], axis=0)

    def lo(w):
        return pltpu.bitcast(w << 16, f32)

    def hi(w):
        return pltpu.bitcast(w & jnp.uint32(0xFFFF0000), f32)

    def FU(i, c):
        base = i * BLK
        hb = base // 2
        ls = pl.ds(c * 128, 128)
        kf[c, pl.ds(8 + hb, BLK // 2), :] = _pk(k_v[pl.ds(base, BLK), ls])
        vf[c, pl.ds(hb, BLK // 2), :] = _pk(v_v[pl.ds(base, BLK), ls])
        kw = {o: kf[c, pl.ds(8 + hb + o, 128, stride=2), :] for o in (-2, -1, 0, 1)}
        Ks = {-3: hi(kw[-2]), -2: lo(kw[-1]), -1: hi(kw[-1]), 0: lo(kw[0]), 1: hi(kw[0]),
              2: lo(kw[1]), 3: hi(kw[1])}
        vw = [vf[c, pl.ds(hb + o, 128, stride=2), :] for o in (0, 1)]
        Vs = [lo(vw[0]), hi(vw[0]), lo(vw[1]), hi(vw[1])]
        wc = [cw[c, j:j + 1, :] for j in range(4)]
        T = []
        for n2 in range(N2):
            ks = (Ks[n2] * wc[0] + Ks[n2 - 1] * wc[1]) + (Ks[n2 - 2] * wc[2] + Ks[n2 - 3] * wc[3])
            u = (ks * Vs[n2]).astype(bf16)
            T.append(jnp.dot(_upk(F_v[n2]), u, preferred_element_type=f32))
        for g in range(16):
            U = _fft4([split(T[n2], g) for n2 in range(N2)], False)
            for k2 in range(N2):
                Us[c, i * N2 + k2, 16 * g:16 * g + 16, :] = join(U[k2])

    def FH(i, c):
        base = i * BLK
        hT[c, pl.ds(base, BLK), :] = h_v[pl.ds(c * 128, 128), pl.ds(base, BLK)].astype(f32).T
        T = []
        for n2 in range(N2):
            hh = hT[c, pl.ds(base + n2, 128, stride=N2), :].astype(bf16)
            T.append(jnp.dot(_upk(F_v[n2]), hh, preferred_element_type=f32))
        for g in range(16):
            Hj = _fft4([split(T[n2], g) for n2 in range(N2)], False)
            if i == 0:
                Hj = [(re + cw[c, 4:5, :], im) for re, im in Hj]
            for k2 in range(N2):
                Hs[c, i * N2 + k2, 16 * g:16 * g + 16, :] = join(Hj[k2])

    def INV(j, c, half):
        Zs = [[] for _ in range(N2)]
        for g in range(8 * half, 8 * half + 8):
            def ld(ref, s):
                t = ref[c, s, 16 * g:16 * g + 16, :]
                return (t[0:8], t[8:16])
            C = []
            for k2 in range(N2):
                Hm = [ld(Hs, m * N2 + k2) for m in range(j + 1)]
                cr = ci = None
                for m in range(j + 1):
                    gr, gi = Hm[m]
                    if m > 0:
                        pr_, pi_ = Hm[m - 1]
                        if half == 0:
                            gr, gi = gr - pi_, gi + pr_
                        else:
                            gr, gi = gr + pi_, gi - pr_
                    ur, ui = ld(Us, (j - m) * N2 + k2)
                    pr = ur * gr - ui * gi
                    pi = ur * gi + ui * gr
                    cr = pr if cr is None else cr + pr
                    ci = pi if ci is None else ci + pi
                C.append((cr, ci))
            Z = _fft4(C, True)
            for n2 in range(N2):
                Zs[n2].append(join(Z[n2]).astype(bf16))
        dst = ya_s if half == 0 else y_s
        for n2 in range(N2):
            dst[c, pl.ds(j * BLK + n2, 128, stride=N2), :] = jnp.dot(
                _upk(FT_v[n2, half]), jnp.concatenate(Zs[n2], axis=0), preferred_element_type=f32)

    def wprep(which, dst):
        pr = lax.broadcasted_iota(jnp.int32, (128, 128), 0)
        pc = lax.broadcasted_iota(jnp.int32, (128, 128), 1)
        perm = jnp.where(pc == (pr % 8) * DH + pr // 8, 1.0, 0.0).astype(bf16)
        outs = []
        for a in range(4):
            wa = wqkv_v[:, which * D + 128 * a:which * D + 128 * (a + 1)]
            outs.append(lax.dot_general(perm, wa, NT, preferred_element_type=f32))
        for dh in range(DH):
            blk = jnp.concatenate([outs[a][8 * dh:8 * dh + 8, :] for a in range(4)], axis=0)
            blk = blk.astype(bf16)
            for c in range(4):
                dst[c, dh * H // 2:(dh + 1) * H // 2, :] = _pk(blk[:, c * 128:(c + 1) * 128])

    def a_layer(src, t, slot=None):
        slot = t if slot is None else slot
        rows = _ds(t, TS, 0, TS)
        x = src[rows, :].astype(f32)
        y = _cat(y_s, rows)
        if src is q_v:
            y = y + _cat(ya_s, rows)
            for c in range(4):
                y_s[c, rows, :] = y[:, c * 128:(c + 1) * 128]
        x = x + _ln(x) * y
        x_s[rows, :] = x
        xn = _ln(x).astype(bf16)
        for c in range(4):
            xn_s[c, pl.ds(slot * (TS // 2), TS // 2), :] = _pk(xn[:, c * 128:(c + 1) * 128])

    def KT(t, c, slot=None):
        slot = t if slot is None else slot
        xn = _catp(xn_s, pl.ds(slot * (TS // 2) + c * 64, 64))
        kT = lax.dot_general(_catp(wkT), xn, NT, preferred_element_type=f32)
        pkT = _phi(kT)
        if isinstance(t, int) and t == 0 and c == 0:
            z_s[...] = pkT
        else:
            z_s[...] += pkT
        pk_s[c, 0:D // 2, :] = _pk(pkT.astype(bf16))

    def PP(t, c, slot=None):
        slot = t if slot is None else slot
        pp = jnp.dot(_catp(pk_s), _upk(xn_s[c, pl.ds(slot * (TS // 2), TS // 2), :]),
                     preferred_element_type=f32)
        if isinstance(t, int) and t == 0:
            P_s[c, 0:D, :] = pp
        else:
            P_s[c, 0:D, :] += pp

    def QQ(t, c, slot=None):
        slot = t if slot is None else slot
        qq = lax.dot_general(
            _catp(xn_s, pl.ds(slot * (TS // 2), TS // 2)), _catp(wqT, pl.ds(c * 64, 64)), NT,
            preferred_element_type=f32)
        pq_s[c, _ds(t, TS, 0, TS), :] = _phi(qq)

    def mid_kv():
        row = lax.broadcasted_iota(jnp.int32, (128, 128), 0) % 8
        col = lax.broadcasted_iota(jnp.int32, (128, 128), 1) // DH
        mask = row == col
        kvs = []
        for j in range(4):
            Pj = jnp.concatenate(
                [_cat(P_s, pl.ds(dh * H + 8 * j, 8)) for dh in range(DH)], axis=0)
            kv = jnp.dot(Pj.astype(bf16), wqkv_v[:, 2 * D + 128 * j:2 * D + 128 * (j + 1)],
                         preferred_element_type=f32)
            kvs.append(jnp.where(mask, kv, 0.0).astype(bf16))
        return kvs

    def mid_m(kvs):
        Ms = [jnp.dot(kvs[j], wo_v[128 * j:128 * (j + 1), :], preferred_element_type=f32)
              for j in range(4)]
        for dh in range(DH):
            blk = jnp.concatenate([Ms[j][8 * dh:8 * dh + 8, :] for j in range(4)], axis=0)
            blk = blk.astype(bf16)
            for c in range(4):
                M_s[c, dh * H // 2:(dh + 1) * H // 2, :] = _pk(blk[:, c * 128:(c + 1) * 128])

    def zrow():
        zr_s[...] = jnp.sum(z_s[...].T, axis=0, keepdims=True)

    def PQN(r0, n):
        rows = pl.ds(r0, n)
        z = zr_s[...]
        pq = [pq_s[c, rows, :] for c in range(4)]
        tt = [pq[c] * z[:, c * 128:(c + 1) * 128] for c in range(4)]
        tt = (tt[0] + tt[1]) + (tt[2] + tt[3])
        tt = tt + pltpu.roll(tt, 32, 1)
        tt = tt + pltpu.roll(tt, 64, 1)
        r = 1.0 / (tt + 1e-6)
        return [(pq[c] * r).astype(bf16) for c in range(4)]

    def OUT(r0, n, pqn=None):
        if pqn is None:
            pqn = _catp(pn_s, pl.ds((r0 - LAST * TS) // 2, n // 2))
        else:
            pqn = jnp.concatenate(pqn, axis=1)
        return x_s[pl.ds(r0, n), :] + jnp.dot(pqn, _catp(M_s), preferred_element_type=f32)

    pieces = [(t * TS, TS) for t in range(LAST)] + [
        (LAST * TS, 256), (LAST * TS + 256, 128), (LAST * TS + 384, 128)]

    def out_copy(i):
        rows = pl.ds(*pieces[i])
        return pltpu.make_async_copy(o_v.at[rows], o_hbm.at[rows], osems.at[i])

    ops = {"H": FH, "U": FU, "a": lambda j, c: INV(j, c, 0), "b": lambda j, c: INV(j, c, 1),
           "K": KT, "P": PP, "Q": QQ}
    for name, waits, toks in SCHED:
        if waits:
            wait(*waits.split())
        else:
            barrier()
        for tok in toks.split():
            if tok == "wk":
                wprep(1, wkT)
            elif tok == "wq":
                wprep(0, wqT)
            elif tok[0] == "L":
                a_layer(q_v, int(tok[1]))
            else:
                ops[tok[0]](int(tok[1]), int(tok[2]))

    def layer(l, carry):
        for c in range(4):
            PP(LAST, c)
        for c in range(4):
            QQ(LAST, c)
        mid_m(mid_kv())
        zrow()
        P_s[...] = jnp.zeros_like(P_s)
        for t in range(LAST):
            res = OUT(t * TS, TS, PQN(t * TS, TS))
            x_s[pl.ds(t * TS, TS), :] = res
            o_v[pl.ds(t * TS, TS), :] = res.astype(bf16)
            if t == 0:
                staged = PQN(LAST * TS, TS)
                for c in range(4):
                    pn_s[c, 0:TS // 2, :] = _pk(staged[c])
            out_copy(t).start()

        @pl.when(l == 0)
        def _():
            a_layer(x_s, 0, LAST)
            for tok in "O0 O1 O2 K0 K1 K2 K3 O3".split():
                c = int(tok[1])
                if tok[0] == "O":
                    r0 = LAST * TS + c * 128
                    x_s[pl.ds(r0, 128), :] = OUT(r0, 128)
                else:
                    KT(0, c, LAST)
            for t in range(LAST):
                out_copy(t).wait()

            def tile(t, carry2):
                for c in range(4):
                    PP(t - 1, c, LAST)
                    QQ(t - 1, c, LAST)
                a_layer(x_s, t, LAST)
                for c in range(4):
                    KT(t, c, LAST)
                return carry2
            lax.fori_loop(1, NT_, tile, 0)
        return carry

    lax.fori_loop(0, 2, layer, 0)

    for i in range(LAST, len(pieces)):
        r0, n = pieces[i]
        o_v[pl.ds(r0, n), :] = OUT(r0, n).astype(bf16)
        out_copy(i).start()
    for i in range(len(pieces)):
        out_copy(i).wait()


@jax.jit
def pallas_interleave_layers__ssm_conv_h3__linear_attn_block__prompt_kernel(
        A_q, A_k, A_v, A_shift_k, A_ssm_k, A_ssm_D, B_x, B_wqkv, B_wo):
    anyspec = pl.BlockSpec(memory_space=pl.ANY)
    out = pl.pallas_call(
        kernel,
        out_shape=jax.ShapeDtypeStruct((S, D), bf16),
        in_specs=[anyspec] * 8,
        out_specs=anyspec,
        scratch_shapes=[
            pltpu.VMEM((S, D), bf16),
            pltpu.VMEM((S, D), bf16),
            pltpu.VMEM((S, D), bf16),
            pltpu.VMEM((4, D), bf16),
            pltpu.VMEM((D, S), bf16),
            pltpu.VMEM((4, 128), bf16),
            pltpu.VMEM((D, 3 * D), bf16),
            pltpu.VMEM((D, D), bf16),
            pltpu.VMEM((S, D), bf16),
            pltpu.VMEM((N2, 128, 128), u32),
            pltpu.VMEM((N2, 2, 64, 128), u32),
            pltpu.VMEM((4, S // 2 + 16, 128), u32),
            pltpu.VMEM((4, S // 2 + 8, 128), u32),
            pltpu.VMEM((4, S + 8, 128), f32),
            pltpu.VMEM((4, 16, 256, 128), f32),
            pltpu.VMEM((4, 16, 256, 128), f32),
            pltpu.VMEM((4, S + 8, 128), f32),
            pltpu.VMEM((4, S + 8, 128), f32),
            pltpu.VMEM((S, D), f32),
            pltpu.VMEM((4, S // 2 + 8, 128), u32),
            pltpu.VMEM((4, D // 2 + 8, 128), u32),
            pltpu.VMEM((4, S + 8, 128), f32),
            pltpu.VMEM((4, D + 8, 128), f32),
            pltpu.VMEM((D, 128), f32),
            pltpu.VMEM((1, D), f32),
            pltpu.VMEM((4, D // 2 + 8, 128), u32),
            pltpu.VMEM((4, D // 2 + 8, 128), u32),
            pltpu.VMEM((4, D // 2 + 8, 128), u32),
            pltpu.VMEM((4, 8, 128), f32),
            pltpu.VMEM((4, TS // 2 + 8, 128), u32),
            pltpu.SemaphoreType.DMA((32,)),
            pltpu.SemaphoreType.DMA((8,)),
            pltpu.SemaphoreType.REGULAR,
        ],
        compiler_params=pltpu.CompilerParams(vmem_limit_bytes=110 * 1024 * 1024),
    )(A_q.reshape(S, D), A_k.reshape(S, D), A_v.reshape(S, D), A_shift_k.T, A_ssm_k,
      A_ssm_D.reshape(4, 128), B_wqkv, B_wo)
    return out.reshape(1, S, D)
```
